```python
import os as _os
_os.environ.setdefault('JAX_PLATFORMS', 'cpu')
import jax
import jax.numpy as jnp

def _softmax(x, axis=-1):
    return jax.nn.softmax(x, axis=axis)

def _gelu(x):
    return jax.nn.gelu(x, approximate=True)

def _silu(x):
    return jax.nn.silu(x)

def _sigmoid(x):
    return jax.nn.sigmoid(x)

def _layernorm(x, axis=-1, eps=1e-05):
    m = jnp.mean(x, axis=axis, keepdims=True)
    v = jnp.var(x, axis=axis, keepdims=True)
    return (x - m) / jnp.sqrt(v + eps)

def _scatter_add(tgt, idx, src, axis=0):
    return tgt.at[idx].add(src)

def _segment_sum(src, seg, n):
    return jax.ops.segment_sum(src, seg, n)

class _Rng:

    def __init__(self, key):
        self._k = key

    def _next(self):
        self._k, sub = jax.random.split(self._k)
        return sub

    def normal(self, shape):
        return jax.random.normal(self._next(), shape, dtype=jnp.bfloat16)

    def randint(self, lo, hi, shape):
        return jax.random.randint(self._next(), shape, lo, hi, dtype=jnp.int32)

    def uniform(self, shape, lo=0.0, hi=1.0):
        return jax.random.uniform(self._next(), shape, jnp.bfloat16, lo, hi)

    def permutation(self, n):
        return jax.random.permutation(self._next(), n)
kernel_name = 'gated_mix__memory_aug_recurrent_mem_tr__glu_gated_geglu__prompt'

def setup_inputs():
    _rng = _Rng(jax.random.key(int.from_bytes(__import__("os").urandom(4), "little")))
    _w = lambda a: (lambda t: t.astype(jnp.bfloat16) if jnp.issubdtype(t.dtype, jnp.floating) else t)(jnp.asarray(a))

    def _A_setup():
        B, S, Dm = (1, 2048, 640)
        H, Dh = (32, 128)
        M, seg = (8, 32)
        seg = min(seg, S)
        S = S // seg * seg
        return {'x': _w((lambda *s: _rng.normal(s) * 0.05)(B, S, Dm)), 'mem0': _w((lambda *s: _rng.normal(s) * 0.4)(B, M, Dm)), 'Wq': _w((lambda *s: _rng.normal(s) * 3.2)(Dm, H, Dh) * Dm ** (-0.5)), 'Wk': _w((lambda *s: _rng.normal(s) * 3.2)(Dm, H, Dh) * Dm ** (-0.5)), 'Wv': _w((lambda *s: _rng.normal(s) * 0.4)(Dm, H, Dh) * Dm ** (-0.5)), 'Wo': _w((lambda *s: _rng.normal(s) * 0.4)(H, Dh, Dm) * (H * Dh) ** (-0.5)), 'seg_len': seg}
    _A_in = _A_setup()

    def _B_setup():
        B, S, Dm, Df = (1, 2048, 640, 1728)
        return {'x': _w((lambda *s: _rng.normal(s) * 0.05)(B, S, Dm)), 'w_gate': _w((lambda *s: _rng.normal(s) * 1.6)(Dm, Df) * Dm ** (-0.5)), 'w_up': _w((lambda *s: _rng.normal(s) * 1.6)(Dm, Df) * Dm ** (-0.5)), 'w_down': _w((lambda *s: _rng.normal(s) * 1.6)(Df, Dm) * Df ** (-0.5))}
    _B_in = _B_setup()
    return {'A_x': _A_in['x'], 'A_mem0': _A_in['mem0'], 'A_Wq': _A_in['Wq'], 'A_Wk': _A_in['Wk'], 'A_Wv': _A_in['Wv'], 'A_Wo': _A_in['Wo'], 'A_seg_len': _A_in['seg_len'], 'B_x': _B_in['x'], 'B_w_gate': _B_in['w_gate'], 'B_w_up': _B_in['w_up'], 'B_w_down': _B_in['w_down'], 'gate_w': _w((lambda *s: _rng.normal(s) * 0.05)(640) * 16.0)}

def reference(A_x, A_mem0, A_Wq, A_Wk, A_Wv, A_Wo, A_seg_len, B_x, B_w_gate, B_w_up, B_w_down, gate_w):

    def _A_ref(x, mem0, Wq, Wk, Wv, Wo, seg_len):
        B, S, Dm = x.shape
        H, Dh = (Wq.shape[1], Wq.shape[2])
        M = mem0.shape[1]
        scale = Dh ** (-0.5)
        n_seg = S // seg_len
        L = M + seg_len
        idx = jnp.arange(L)
        mask = (idx[:, None] < M) | (idx[:, None] >= idx[None, :])
        mem = mem0
        outs = []
        for s in range(n_seg):
            xs = x[:, s * seg_len:(s + 1) * seg_len, :].copy()
            h = jnp.concatenate([mem, xs], axis=1)
            q = jnp.einsum('btd,dhe->bhte', h, Wq)
            k = jnp.einsum('btd,dhe->bhte', h, Wk)
            v = jnp.einsum('btd,dhe->bhte', h, Wv)
            scores = jnp.einsum('bhqe,bhke->bhqk', q, k) * scale
            scores = jnp.where(mask[None, None], scores, -1000000000.0)
            p = _softmax(scores, axis=-1)
            o = jnp.einsum('bhqk,bhke->bhqe', p, v)
            o = jnp.einsum('bhte,hed->btd', o, Wo)
            mem = o[:, :M, :].copy()
            outs.append(o[:, M:, :])
        return jnp.concatenate(outs, axis=1)

    def _B_ref(x, w_gate, w_up, w_down):
        g = jnp.einsum('bsd,df->bsf', x, w_gate)
        u = jnp.einsum('bsd,df->bsf', x, w_up)
        h = _gelu(g) * u
        return jnp.einsum('bsf,fd->bsd', h, w_down)
    x = A_x
    g = _sigmoid((x * gate_w).sum(-1, keepdims=True))
    a = _A_ref(x, A_mem0, A_Wq, A_Wk, A_Wv, A_Wo, A_seg_len)
    b = _B_ref(x, B_w_gate, B_w_up, B_w_down)
    return g * a + (1 - g) * b
```

```python
import jax
import jax.numpy as jnp
from jax import lax
import jax.experimental.pallas as pl
import jax.experimental.pallas.tpu as pltpu

_F32 = jnp.float32
_BF16 = jnp.bfloat16


def _mm(a, b):
    return lax.dot_general(a, b, (((1,), (0,)), ((), ())), preferred_element_type=_F32)


def _mm_nt(a, b):
    return lax.dot_general(a, b, (((1,), (1,)), ((), ())), preferred_element_type=_F32)


def _make_kernel(S, D, H, E, M, seg, F, glu_rows):
    n_seg = S // seg
    L = seg + M
    scale = float(E) ** -0.5

    def kernel(x_ref, mem0_ref, gw_ref, wg_ref, wu_ref, wd_ref,
               wq_hbm, wk_hbm, wv_hbm, wo_hbm,
               o_ref,
               raw_ref, wqkv_ref, wo_ref, b_ref, sems):
        copies = [pltpu.make_async_copy(w, raw_ref.at[i], sems.at[i])
                  for i, w in enumerate((wq_hbm, wk_hbm, wv_hbm))]
        copies.append(pltpu.make_async_copy(wo_hbm, wo_ref, sems.at[3]))
        for c in copies:
            c.start()

        def glu_body(i, carry):
            r0 = pl.multiple_of(i * glu_rows, glu_rows)
            xb = x_ref[pl.ds(r0, glu_rows), :]
            g = _mm(xb, wg_ref[...])
            u = _mm(xb, wu_ref[...])
            hid = (jax.nn.gelu(g, approximate=True) * u).astype(_BF16)
            b_ref[pl.ds(r0, glu_rows), :] = _mm(hid, wd_ref[...])
            return carry

        lax.fori_loop(0, S // glu_rows, glu_body, 0)

        for i in range(3):
            copies[i].wait()
            w32 = raw_ref.at[i].bitcast(jnp.uint32)
            for j in range(H // 2):
                w = w32[pl.ds(j, D, stride=H // 2), :]
                lo = pltpu.bitcast(w << 16, _F32).astype(_BF16)
                hi = pltpu.bitcast(w & jnp.uint32(0xFFFF0000), _F32).astype(_BF16)
                wqkv_ref[2 * j, :, i * E:(i + 1) * E] = lo
                wqkv_ref[2 * j + 1, :, i * E:(i + 1) * E] = hi
        copies[3].wait()

        row = lax.broadcasted_iota(jnp.int32, (L, L), 0)
        col = lax.broadcasted_iota(jnp.int32, (L, L), 1)
        allowed = (row >= seg) | (col >= seg) | (col <= row)
        gw = gw_ref[...].astype(_F32)

        def seg_body(s, mem):
            r0 = pl.multiple_of(s * seg, seg)
            xs = x_ref[pl.ds(r0, seg), :].astype(_F32)
            hcat = jnp.concatenate([xs, mem], axis=0)
            acc = None
            for h in range(H):
                qkv = _mm(hcat, wqkv_ref[h])
                q = qkv[:, 0:E] * scale
                k = qkv[:, E:2 * E].astype(_BF16)
                v = qkv[:, 2 * E:3 * E].astype(_BF16)
                sc = jnp.where(allowed, _mm_nt(q, k), -1000000000.0)
                e = jnp.exp(sc - jnp.max(sc, axis=-1, keepdims=True))
                p = e / jnp.sum(e, axis=-1, keepdims=True)
                o = _mm(p, v)
                c = _mm(o, wo_ref[h * E:(h + 1) * E, :])
                acc = c if acc is None else acc + c
            gate = jax.nn.sigmoid(jnp.sum(xs * gw, axis=-1, keepdims=True))
            out = gate * acc[0:seg] + (1.0 - gate) * b_ref[pl.ds(r0, seg), :]
            o_ref[pl.ds(r0, seg), :] = out.astype(o_ref.dtype)
            return acc[seg:L].astype(_BF16).astype(_F32)

        lax.fori_loop(0, n_seg, seg_body, mem0_ref[...].astype(_F32))

    return kernel


@jax.jit(static_argnames=("A_seg_len",))
def pallas_gated_mix__memory_aug_recurrent_mem_tr__glu_gated_geglu__prompt_kernel(
    A_x, A_mem0, A_Wq, A_Wk, A_Wv, A_Wo, A_seg_len,
    B_x, B_w_gate, B_w_up, B_w_down, gate_w,
):
    del B_x
    B, S, D = A_x.shape
    _, H, E = A_Wq.shape
    M = A_mem0.shape[1]
    F = B_w_gate.shape[1]
    seg = int(A_seg_len)
    assert B == 1 and S % seg == 0

    kernel = _make_kernel(S, D, H, E, M, seg, F, glu_rows=256)
    vmem = pl.BlockSpec(memory_space=pltpu.VMEM)
    hbm = pl.BlockSpec(memory_space=pl.ANY)
    out = pl.pallas_call(
        kernel,
        out_shape=jax.ShapeDtypeStruct((S, D), A_x.dtype),
        in_specs=[vmem] * 6 + [hbm] * 4,
        out_specs=vmem,
        scratch_shapes=[
            pltpu.VMEM((3, D * H, E), _BF16),
            pltpu.VMEM((H, D, 3 * E), _BF16),
            pltpu.VMEM((H * E, D), _BF16),
            pltpu.VMEM((S, D), _F32),
            pltpu.SemaphoreType.DMA((4,)),
        ],
        compiler_params=pltpu.CompilerParams(vmem_limit_bytes=100 * 1024 * 1024),
    )(
        A_x.reshape(S, D), A_mem0.reshape(M, D), gate_w.reshape(1, D),
        B_w_gate, B_w_up, B_w_down,
        A_Wq.reshape(D * H, E), A_Wk.reshape(D * H, E), A_Wv.reshape(D * H, E),
        A_Wo.reshape(H * E, D),
    )
    return out.reshape(B, S, D)
```

```python
import jax
import jax.numpy as jnp
from jax import lax
import jax.experimental.pallas as pl
import jax.experimental.pallas.tpu as pltpu

_F32 = jnp.float32
_BF16 = jnp.bfloat16


def _mm(a, b):
    return lax.dot_general(a, b, (((1,), (0,)), ((), ())), preferred_element_type=_F32)


def _mm_nt(a, b):
    return lax.dot_general(a, b, (((1,), (1,)), ((), ())), preferred_element_type=_F32)


def _make_kernel(S, D, H, E, M, seg, F, glu_rows):
    n_seg = S // seg
    L = seg + M
    scale = float(E) ** -0.5

    def kernel(x_ref, mem0_ref, gw_ref, wg_ref, wu_ref, wd_ref,
               wq_hbm, wk_hbm, wv_hbm, wo_hbm,
               o_ref,
               raw_ref, wqkv_ref, wo_ref, b_ref, sems):
        copies = [pltpu.make_async_copy(w, raw_ref.at[i], sems.at[i])
                  for i, w in enumerate((wq_hbm, wk_hbm, wv_hbm))]
        copies.append(pltpu.make_async_copy(wo_hbm, wo_ref, sems.at[3]))
        for c in copies:
            c.start()

        def glu_body(i, carry):
            r0 = pl.multiple_of(i * glu_rows, glu_rows)
            xb = x_ref[pl.ds(r0, glu_rows), :]
            g = _mm(xb, wg_ref[...])
            u = _mm(xb, wu_ref[...])
            hid = (jax.nn.gelu(g, approximate=True) * u).astype(_BF16)
            b_ref[pl.ds(r0, glu_rows), :] = _mm(hid, wd_ref[...])
            return carry

        lax.fori_loop(0, S // glu_rows, glu_body, 0)

        for i in range(3):
            copies[i].wait()
            w32 = raw_ref.at[i].bitcast(jnp.uint32)
            for j in range(H // 2):
                w = w32[pl.ds(j, D, stride=H // 2), :]
                lo = pltpu.bitcast(w << 16, _F32).astype(_BF16)
                hi = pltpu.bitcast(w & jnp.uint32(0xFFFF0000), _F32).astype(_BF16)
                wqkv_ref[2 * j, :, i * E:(i + 1) * E] = lo
                wqkv_ref[2 * j + 1, :, i * E:(i + 1) * E] = hi
        copies[3].wait()

        row = lax.broadcasted_iota(jnp.int32, (L, L), 0)
        col = lax.broadcasted_iota(jnp.int32, (L, L), 1)
        allowed = (row >= seg) | (col >= seg) | (col <= row)
        gw = gw_ref[...].astype(_F32)

        def seg_body(s, mem):
            r0 = pl.multiple_of(s * seg, seg)
            xs = x_ref[pl.ds(r0, seg), :].astype(_F32)
            hcat = jnp.concatenate([xs, mem], axis=0)
            qkv = [_mm(hcat, wqkv_ref[h]) for h in range(H)]
            sc = [_mm_nt(t[:, 0:E] * scale, t[:, E:2 * E].astype(_BF16)) for t in qkv]
            ps = []
            for t in sc:
                t = jnp.where(allowed, t, -1000000000.0)
                e = jnp.exp(t - jnp.max(t, axis=-1, keepdims=True))
                ps.append(e / jnp.sum(e, axis=-1, keepdims=True))
            os_ = [_mm(p, t[:, 2 * E:3 * E].astype(_BF16)) for p, t in zip(ps, qkv)]
            acc = _mm(jnp.concatenate(os_, axis=1), wo_ref[...])
            gate = jax.nn.sigmoid(jnp.sum(xs * gw, axis=-1, keepdims=True))
            out = gate * acc[0:seg] + (1.0 - gate) * b_ref[pl.ds(r0, seg), :]
            o_ref[pl.ds(r0, seg), :] = out.astype(o_ref.dtype)
            return acc[seg:L].astype(_BF16).astype(_F32)

        lax.fori_loop(0, n_seg, seg_body, mem0_ref[...].astype(_F32))

    return kernel


@jax.jit(static_argnames=("A_seg_len",))
def pallas_gated_mix__memory_aug_recurrent_mem_tr__glu_gated_geglu__prompt_kernel(
    A_x, A_mem0, A_Wq, A_Wk, A_Wv, A_Wo, A_seg_len,
    B_x, B_w_gate, B_w_up, B_w_down, gate_w,
):
    del B_x
    B, S, D = A_x.shape
    _, H, E = A_Wq.shape
    M = A_mem0.shape[1]
    F = B_w_gate.shape[1]
    seg = int(A_seg_len)
    assert B == 1 and S % seg == 0

    kernel = _make_kernel(S, D, H, E, M, seg, F, glu_rows=256)
    vmem = pl.BlockSpec(memory_space=pltpu.VMEM)
    hbm = pl.BlockSpec(memory_space=pl.ANY)
    out = pl.pallas_call(
        kernel,
        out_shape=jax.ShapeDtypeStruct((S, D), A_x.dtype),
        in_specs=[vmem] * 6 + [hbm] * 4,
        out_specs=vmem,
        scratch_shapes=[
            pltpu.VMEM((3, D * H, E), _BF16),
            pltpu.VMEM((H, D, 3 * E), _BF16),
            pltpu.VMEM((H * E, D), _BF16),
            pltpu.VMEM((S, D), _F32),
            pltpu.SemaphoreType.DMA((4,)),
        ],
        compiler_params=pltpu.CompilerParams(vmem_limit_bytes=100 * 1024 * 1024),
    )(
        A_x.reshape(S, D), A_mem0.reshape(M, D), gate_w.reshape(1, D),
        B_w_gate, B_w_up, B_w_down,
        A_Wq.reshape(D * H, E), A_Wk.reshape(D * H, E), A_Wv.reshape(D * H, E),
        A_Wo.reshape(H * E, D),
    )
    return out.reshape(B, S, D)
```

```python
import jax
import jax.numpy as jnp
from jax import lax
import jax.experimental.pallas as pl
import jax.experimental.pallas.tpu as pltpu

_F32 = jnp.float32
_BF16 = jnp.bfloat16
_GROUPS = (4,) * 8
_SK = 4
_OUT_CHUNKS = 8


def _mm(a, b):
    return lax.dot_general(a, b, (((1,), (0,)), ((), ())), preferred_element_type=_F32)


def _mm_nt(a, b):
    return lax.dot_general(a, b, (((1,), (1,)), ((), ())), preferred_element_type=_F32)


def _make_kernel(S, D, H, E, M, seg, F, glu_rows):
    n_seg = S // seg
    L = seg + M
    scale = float(E) ** -0.5

    def kernel(mem0_ref, gw_ref, x_hbm, wg_hbm, wu_hbm, wd_hbm,
               wq_hbm, wk_hbm, wv_hbm, wo_hbm,
               o_hbm,
               x_ref, wg_ref, wu_ref, wd_ref, o_ref,
               raw_ref, wqkv_ref, wo_ref, b_ref, sems, osems):
        n_glu = S // glu_rows
        srcs = (x_hbm.at[pl.ds(0, glu_rows)], wg_hbm, wu_hbm, wd_hbm,
                x_hbm.at[pl.ds(glu_rows, S - glu_rows)], wq_hbm, wk_hbm, wv_hbm, wo_hbm)
        dsts = (x_ref.at[pl.ds(0, glu_rows)], wg_ref, wu_ref, wd_ref,
                x_ref.at[pl.ds(glu_rows, S - glu_rows)],
                raw_ref.at[0], raw_ref.at[1], raw_ref.at[2], wo_ref)
        copies = [pltpu.make_async_copy(a, b, sems.at[i])
                  for i, (a, b) in enumerate(zip(srcs, dsts))]
        for c in copies[:5]:
            c.start()

        def glu(i, first=False):
            r0 = pl.multiple_of(i * glu_rows, glu_rows)
            if first:
                copies[0].wait()
                copies[1].wait()
            xb = x_ref[pl.ds(r0, glu_rows), :]
            g = _mm_nt(xb, wg_ref[...])
            if first:
                copies[2].wait()
                for c in copies[5:]:
                    c.start()
            u = _mm_nt(xb, wu_ref[...])
            hid = (jax.nn.gelu(g, approximate=True) * u).astype(_BF16)
            if first:
                copies[3].wait()
            b_ref[pl.ds(r0, glu_rows), :] = _mm(hid, wd_ref[...])

        n_rel = n_glu // 2
        dc = D // n_rel

        def relayout(c):
            d0 = pl.multiple_of(c * dc, dc)
            for i in range(3):
                w32 = raw_ref.at[i, pl.ds(pl.multiple_of(c * (dc * H), dc * H), dc * H)]
                w32 = w32.bitcast(jnp.uint32)
                for j in range(H // 2):
                    w = w32[pl.ds(j, dc, stride=H // 2), :]
                    lo = pltpu.bitcast(w << 16, _F32).astype(_BF16)
                    hi = pltpu.bitcast(w & jnp.uint32(0xFFFF0000), _F32).astype(_BF16)
                    wqkv_ref[2 * j, pl.ds(d0, dc), i * E:(i + 1) * E] = lo
                    wqkv_ref[2 * j + 1, pl.ds(d0, dc), i * E:(i + 1) * E] = hi

        glu(0, first=True)
        copies[4].wait()

        def body_a(i, carry):
            glu(i)
            return carry

        lax.fori_loop(1, n_glu - n_rel, body_a, 0)
        for c in copies[5:]:
            c.wait()

        def body_b(c, carry):
            glu(c + (n_glu - n_rel))
            relayout(c)
            return carry

        lax.fori_loop(0, n_rel, body_b, 0)

        row = lax.broadcasted_iota(jnp.int32, (L, L), 0)
        col = lax.broadcasted_iota(jnp.int32, (L, L), 1)
        allowed = (row >= seg) | (col >= seg) | (col <= row)
        gw = gw_ref[...].astype(_F32)

        def seg_body(s, mem):
            r0 = pl.multiple_of(s * seg, seg)
            xs = x_ref[pl.ds(r0, seg), :].astype(_F32)
            hcat = jnp.concatenate([xs, mem], axis=0)
            qkv, sc, ps, os_ = {}, {}, {}, {}
            acc = None
            inv = {}
            bounds = [0]
            for n in _GROUPS:
                bounds.append(bounds[-1] + n)
            assert bounds[-1] == H
            grp = lambda t: range(bounds[t], bounds[t + 1]) if 0 <= t < len(_GROUPS) else ()
            for t in range(len(_GROUPS) + _SK):
                for h in grp(t):
                    qkv[h] = _mm(hcat, wqkv_ref[h])
                for h in grp(t - 1):
                    z = qkv[h]
                    z = _mm_nt(z[:, 0:E] * scale, z[:, E:2 * E].astype(_BF16))
                    z = jnp.where(allowed, z, -1000000000.0)
                    ps[h] = jnp.exp(z - jnp.max(z, axis=-1, keepdims=True))
                    inv[h] = 1.0 / jnp.sum(ps[h], axis=-1, keepdims=True)
                for h in grp(t - 2):
                    os_[h] = _mm(ps[h], qkv[h][:, 2 * E:3 * E].astype(_BF16)) * inv[h]
                hs = grp(t - _SK)
                if len(hs):
                    c = _mm(jnp.concatenate([os_[h] for h in hs], axis=1),
                            wo_ref[hs[0] * E:(hs[-1] + 1) * E, :])
                    acc = c if acc is None else acc + c
            gate = jax.nn.sigmoid(jnp.sum(xs * gw, axis=-1, keepdims=True))
            out = gate * acc[0:seg] + (1.0 - gate) * b_ref[pl.ds(r0, seg), :]
            o_ref[pl.ds(r0, seg), :] = out.astype(o_ref.dtype)
            return acc[seg:L].astype(_BF16).astype(_F32)

        per = n_seg // _OUT_CHUNKS
        rows = per * seg

        def out_copy(c):
            r = pl.ds(pl.multiple_of(c * rows, rows), rows)
            return pltpu.make_async_copy(o_ref.at[r], o_hbm.at[r], osems.at[c])

        def chunk_body(c, mem):
            mem = lax.fori_loop(c * per, (c + 1) * per, seg_body, mem)
            out_copy(c).start()
            return mem

        lax.fori_loop(0, _OUT_CHUNKS, chunk_body, mem0_ref[...].astype(_F32))
        for c in range(_OUT_CHUNKS):
            out_copy(c).wait()

    return kernel


@jax.jit(static_argnames=("A_seg_len",))
def pallas_gated_mix__memory_aug_recurrent_mem_tr__glu_gated_geglu__prompt_kernel(
    A_x, A_mem0, A_Wq, A_Wk, A_Wv, A_Wo, A_seg_len,
    B_x, B_w_gate, B_w_up, B_w_down, gate_w,
):
    del B_x
    B, S, D = A_x.shape
    _, H, E = A_Wq.shape
    M = A_mem0.shape[1]
    F = B_w_gate.shape[1]
    seg = int(A_seg_len)
    assert B == 1 and S % seg == 0

    kernel = _make_kernel(S, D, H, E, M, seg, F, glu_rows=256)
    vmem = pl.BlockSpec(memory_space=pltpu.VMEM)
    hbm = pl.BlockSpec(memory_space=pl.ANY)
    out = pl.pallas_call(
        kernel,
        out_shape=jax.ShapeDtypeStruct((S, D), A_x.dtype),
        in_specs=[vmem] * 2 + [hbm] * 8,
        out_specs=hbm,
        scratch_shapes=[
            pltpu.VMEM((S, D), _BF16),
            pltpu.VMEM((F, D), _BF16),
            pltpu.VMEM((F, D), _BF16),
            pltpu.VMEM((F, D), _BF16),
            pltpu.VMEM((S, D), A_x.dtype),
            pltpu.VMEM((3, D * H, E), _BF16),
            pltpu.VMEM((H, D, 3 * E), _BF16),
            pltpu.VMEM((H * E, D), _BF16),
            pltpu.VMEM((S, D), _F32),
            pltpu.SemaphoreType.DMA((9,)),
            pltpu.SemaphoreType.DMA((_OUT_CHUNKS,)),
        ],
        compiler_params=pltpu.CompilerParams(vmem_limit_bytes=100 * 1024 * 1024),
    )(
        A_mem0.reshape(M, D), gate_w.reshape(1, D), A_x.reshape(S, D),
        B_w_gate.T, B_w_up.T, B_w_down,
        A_Wq.reshape(D * H, E), A_Wk.reshape(D * H, E), A_Wv.reshape(D * H, E),
        A_Wo.reshape(H * E, D),
    )
    return out.reshape(B, S, D)
```

```python
import jax
import jax.numpy as jnp
from jax import lax
import jax.experimental.pallas as pl
import jax.experimental.pallas.tpu as pltpu

_F32 = jnp.float32
_BF16 = jnp.bfloat16
_GROUPS = (4,) * 8
_SK = 4
_FC = 256
_OUT_CHUNKS = 8


def _mm(a, b):
    return lax.dot_general(a, b, (((1,), (0,)), ((), ())), preferred_element_type=_F32)


def _mm_nt(a, b):
    return lax.dot_general(a, b, (((1,), (1,)), ((), ())), preferred_element_type=_F32)


def _make_kernel(S, D, H, E, M, seg, F, glu_rows):
    n_seg = S // seg
    L = seg + M
    scale = float(E) ** -0.5

    def kernel(mem0_ref, gw_ref, x_hbm, wg_hbm, wu_hbm, wd_hbm,
               wq_hbm, wk_hbm, wv_hbm, wo_hbm,
               o_hbm,
               x_ref, wg_ref, wu_ref, wd_ref, o_ref,
               raw_ref, wqkv_ref, wo_ref, b_ref, sems, osems):
        n_glu = S // glu_rows
        srcs = (x_hbm.at[pl.ds(0, glu_rows)], wg_hbm, wu_hbm, wd_hbm,
                x_hbm.at[pl.ds(glu_rows, S - glu_rows)], wo_hbm)
        dsts = (x_ref.at[pl.ds(0, glu_rows)], wg_ref, wu_ref, wd_ref,
                x_ref.at[pl.ds(glu_rows, S - glu_rows)],
                wo_ref)
        copies = [pltpu.make_async_copy(a, b, sems.at[i])
                  for i, (a, b) in enumerate(zip(srcs, dsts))]
        for i, w in enumerate((wq_hbm, wk_hbm, wv_hbm)):
            w32 = w.bitcast(jnp.uint32)
            copies += [pltpu.make_async_copy(w32.at[:, j, :], raw_ref.at[i, j], sems.at[6 + i])
                       for j in range(H // 2)]
        for c in copies[:2]:
            c.start()

        def glu(i, first=False):
            r0 = pl.multiple_of(i * glu_rows, glu_rows)
            if first:
                copies[0].wait()
                copies[1].wait()
                copies[2].start()
            xb = x_ref[pl.ds(r0, glu_rows), :]
            F0 = F // 128 * 128
            g = _mm_nt(xb, wg_ref[0:F0, :])
            if first:
                copies[2].wait()
                copies[3].start()
            u = _mm_nt(xb, wu_ref[0:F0, :])
            r = _mm_nt(xb, jnp.concatenate([wg_ref[F0:F, :], wu_ref[F0:F, :]], axis=0))
            hid = jnp.concatenate([
                (jax.nn.gelu(g, approximate=True) * u).astype(_BF16),
                (jax.nn.gelu(r[:, 0:F - F0], approximate=True) * r[:, F - F0:]).astype(_BF16)], axis=1)
            if first:
                copies[3].wait()
                for c in copies[4:]:
                    c.start()
            b_ref[pl.ds(r0, glu_rows), :] = _mm(hid, wd_ref[...])

        n_rel = 2
        dc = D // n_rel

        def relayout(c):
            d0 = c * dc
            for i in range(3):
                for j in range(H // 2):
                    w = raw_ref[i, j, pl.ds(d0, dc), :]
                    lo = pltpu.bitcast(w << 16, _F32).astype(_BF16)
                    hi = pltpu.bitcast(w & jnp.uint32(0xFFFF0000), _F32).astype(_BF16)
                    wqkv_ref[3 * (2 * j) + i, pl.ds(d0, dc), :] = lo
                    wqkv_ref[3 * (2 * j + 1) + i, pl.ds(d0, dc), :] = hi
                    yield

        def glu_relayout(i, c):
            pieces = relayout(c)
            r0 = i * glu_rows
            xb = x_ref[pl.ds(r0, glu_rows), :]
            cuts = list(range(0, F, _FC)) + [F]
            per = -(-3 * (H // 2) // (len(cuts) - 1))
            acc = None
            for f0, f1 in zip(cuts[:-1], cuts[1:]):
                g = _mm_nt(xb, wg_ref[f0:f1, :])
                u = _mm_nt(xb, wu_ref[f0:f1, :])
                for _ in range(per):
                    next(pieces, None)
                hid = (jax.nn.gelu(g, approximate=True) * u).astype(_BF16)
                c_ = _mm(hid, wd_ref[f0:f1, :])
                acc = c_ if acc is None else acc + c_
            b_ref[pl.ds(r0, glu_rows), :] = acc

        glu(0, first=True)
        copies[4].wait()

        def body_a(i, carry):
            glu(i)
            return carry

        lax.fori_loop(1, n_glu - n_rel, body_a, 0)
        for c in copies[5:]:
            c.wait()

        for c in range(n_rel):
            glu_relayout(c + (n_glu - n_rel), c)

        row = lax.broadcasted_iota(jnp.int32, (L, L), 0)
        col = lax.broadcasted_iota(jnp.int32, (L, L), 1)
        allowed = (row >= seg) | (col >= seg) | (col <= row)
        gw = gw_ref[...].astype(_F32).reshape(1, D)

        def seg_body(s, mem):
            r0 = pl.multiple_of(s * seg, seg)
            xs = x_ref[pl.ds(r0, seg), :].astype(_F32)
            hcat = jnp.concatenate([xs, mem], axis=0)
            qkv, sc, ps, os_ = {}, {}, {}, {}
            acc = None
            inv = {}
            bounds = [0]
            for n in _GROUPS:
                bounds.append(bounds[-1] + n)
            assert bounds[-1] == H
            grp = lambda t: range(bounds[t], bounds[t + 1]) if 0 <= t < len(_GROUPS) else ()
            for t in range(len(_GROUPS) + _SK):
                for h in grp(t):
                    qkv[h] = _mm(hcat, jnp.concatenate(
                        [wqkv_ref[3 * h + i] for i in range(3)], axis=1))
                for h in grp(t - 1):
                    z = qkv[h]
                    z = _mm_nt(z[:, 0:E] * scale, z[:, E:2 * E].astype(_BF16))
                    z = jnp.where(allowed, z, -1000000000.0)
                    ps[h] = jnp.exp(z - jnp.max(z, axis=-1, keepdims=True))
                    inv[h] = 1.0 / jnp.sum(ps[h], axis=-1, keepdims=True)
                for h in grp(t - 2):
                    os_[h] = _mm(ps[h], qkv[h][:, 2 * E:3 * E].astype(_BF16)) * inv[h]
                hs = grp(t - _SK)
                if len(hs):
                    c = _mm(jnp.concatenate([os_[h] for h in hs], axis=1),
                            wo_ref[hs[0] * E:(hs[-1] + 1) * E, :])
                    acc = c if acc is None else acc + c
            gate = jax.nn.sigmoid(jnp.sum(xs * gw, axis=-1, keepdims=True))
            out = gate * acc[0:seg] + (1.0 - gate) * b_ref[pl.ds(r0, seg), :]
            o_ref[pl.ds(r0, seg), :] = out.astype(o_ref.dtype)
            return acc[seg:L].astype(_BF16).astype(_F32)

        per = n_seg // _OUT_CHUNKS
        rows = per * seg

        def out_copy(c):
            r = pl.ds(pl.multiple_of(c * rows, rows), rows)
            return pltpu.make_async_copy(o_ref.at[r], o_hbm.at[r], osems.at[c])

        def chunk_body(c, mem):
            mem = lax.fori_loop(0, per, lambda j, m: seg_body(c * per + j, m), mem, unroll=2)
            out_copy(c).start()
            return mem

        lax.fori_loop(0, _OUT_CHUNKS, chunk_body, mem0_ref[...].astype(_F32))
        for c in range(_OUT_CHUNKS):
            out_copy(c).wait()

    return kernel


@jax.jit(static_argnames=("A_seg_len",))
def pallas_gated_mix__memory_aug_recurrent_mem_tr__glu_gated_geglu__prompt_kernel(
    A_x, A_mem0, A_Wq, A_Wk, A_Wv, A_Wo, A_seg_len,
    B_x, B_w_gate, B_w_up, B_w_down, gate_w,
):
    del B_x
    B, S, D = A_x.shape
    _, H, E = A_Wq.shape
    M = A_mem0.shape[1]
    F = B_w_gate.shape[1]
    seg = int(A_seg_len)
    assert B == 1 and S % seg == 0

    kernel = _make_kernel(S, D, H, E, M, seg, F, glu_rows=256)
    vmem = pl.BlockSpec(memory_space=pltpu.VMEM)
    hbm = pl.BlockSpec(memory_space=pl.ANY)
    out = pl.pallas_call(
        kernel,
        out_shape=jax.ShapeDtypeStruct((S, D), A_x.dtype),
        in_specs=[vmem] * 2 + [hbm] * 8,
        out_specs=hbm,
        scratch_shapes=[
            pltpu.VMEM((S, D), _BF16),
            pltpu.VMEM((F, D), _BF16),
            pltpu.VMEM((F, D), _BF16),
            pltpu.VMEM((F, D), _BF16),
            pltpu.VMEM((S, D), A_x.dtype),
            pltpu.VMEM((3, H // 2, D, E), jnp.uint32),
            pltpu.VMEM((3 * H, D, E), _BF16),
            pltpu.VMEM((H * E, D), _BF16),
            pltpu.VMEM((S, D), _F32),
            pltpu.SemaphoreType.DMA((9,)),
            pltpu.SemaphoreType.DMA((_OUT_CHUNKS,)),
        ],
        compiler_params=pltpu.CompilerParams(vmem_limit_bytes=100 * 1024 * 1024),
    )(
        A_mem0.reshape(M, D), gate_w, A_x.reshape(S, D),
        B_w_gate.T, B_w_up.T, B_w_down,
        A_Wq, A_Wk, A_Wv,
        A_Wo.reshape(H * E, D),
    )
    return out.reshape(B, S, D)
```
